```python
import os as _os
_os.environ.setdefault("JAX_PLATFORMS", "cpu")
import jax
import jax.numpy as jnp

def _softmax(x, axis=-1):
    return jax.nn.softmax(x, axis=axis)
def _gelu(x):
    return jax.nn.gelu(x, approximate=True)
def _silu(x):
    return jax.nn.silu(x)
def _sigmoid(x):
    return jax.nn.sigmoid(x)
def _layernorm(x, axis=-1, eps=1e-5):
    m = jnp.mean(x, axis=axis, keepdims=True)
    v = jnp.var(x, axis=axis, keepdims=True)
    return (x - m) / jnp.sqrt(v + eps)
def _scatter_add(tgt, idx, src, axis=0):
    return tgt.at[idx].add(src)
def _segment_sum(src, seg, n):
    return jax.ops.segment_sum(src, seg, n)
class _Rng:
    def __init__(self, key):
        self._k = key
    def _next(self):
        self._k, sub = jax.random.split(self._k)
        return sub
    def normal(self, shape):
        return jax.random.normal(self._next(), shape, dtype=jnp.bfloat16)
    def randint(self, lo, hi, shape):
        return jax.random.randint(self._next(), shape, lo, hi, dtype=jnp.int32)
    def uniform(self, shape, lo=0.0, hi=1.0):
        return jax.random.uniform(self._next(), shape, jnp.bfloat16, lo, hi)
    def permutation(self, n):
        return jax.random.permutation(self._next(), n)


kernel_name = 'gated_mix__sliding_block__dense_activation_silu__prompt'

def setup_inputs():
    _rng = _Rng(jax.random.key(int.from_bytes(__import__("os").urandom(4), "little")))
    _w = (lambda a: (lambda t: t.astype(jnp.bfloat16) if jnp.issubdtype(t.dtype, jnp.floating) else t)(jnp.asarray(a)))
    def _A_setup():
        B, S, D = 1, 2048, 640
        return {
            "x": _w((lambda *s: _rng.normal(s) * 0.05)(B, S, D)),
            "wqkv": _w((lambda *s: _rng.normal(s) * 0.4)(D, 3 * D)),
            "wo": _w((lambda *s: _rng.normal(s) * 0.05)(D, D)),
        }
    _A_in = _A_setup()

    def _B_setup():
        B, S, D, F = 1, 2048, 640, 1536
        return {
            "x": _w((lambda *s: _rng.normal(s) * 0.05)(B, S, D)),
            "w1": _w((lambda *s: _rng.normal(s) * 1.6)(D, F) * (D ** -0.5)),
            "w2": _w((lambda *s: _rng.normal(s) * 1.6)(F, D) * (F ** -0.5)),
        }
    _B_in = _B_setup()

    return {
        "A_x": _A_in["x"],
        "A_wqkv": _A_in["wqkv"],
        "A_wo": _A_in["wo"],
        "B_x": _B_in["x"],
        "B_w1": _B_in["w1"],
        "B_w2": _B_in["w2"],
        "gate_w": _w((lambda *s: _rng.normal(s) * 0.05)(640) * 16.0),
    }

def reference(A_x, A_wqkv, A_wo, B_x, B_w1, B_w2, gate_w):
    def _A_ref(x, wqkv, wo):
        B, S, D = x.shape
        H = 32; Dh = D // H; W = 256
        qkv = (lambda x, *d: x.transpose(*d))((x @ wqkv).reshape(B, S, 3, H, Dh), 2, 0, 3, 1, 4)
        q, k, v = qkv[0], qkv[1], qkv[2]
        scores = jnp.einsum("bhqd,bhkd->bhqk", q, k) * (Dh ** -0.5)
        idx = jnp.arange(S)
        mask = (idx[:, None] - idx[None, :] >= 0) & (idx[:, None] - idx[None, :] < W)
        scores = jnp.where(mask[None, None], scores, -1e9)
        p = _softmax(scores, axis=-1)
        o = jnp.einsum("bhqk,bhkd->bhqd", p, v)
        return (lambda x, *d: x.transpose(*d))(o, 0, 2, 1, 3).reshape(B, S, D) @ wo

    def _B_ref(x, w1, w2):
        h = jnp.einsum("bsd,df->bsf", x, w1)
        h = _silu(h)
        out = jnp.einsum("bsf,fd->bsd", h, w2)
        return out

    x = A_x
    g = _sigmoid((x * gate_w).sum(-1, keepdims=True))
    a = _A_ref(x, A_wqkv, A_wo)
    b = _B_ref(x, B_w1, B_w2)
    return g * a + (1 - g) * b
```

```python
import functools
import math

import jax
import jax.numpy as jnp
from jax import lax
from jax.experimental import pallas as pl
from jax.experimental.pallas import tpu as pltpu

S, D, F = 2048, 640, 1536
H, DH, W = 32, 20, 256
BQ = 256
QB = 64
NP = H // 2
NU = BQ // QB
KW = W + QB
VR = 48
NT = 6
NEG = -1e30
QSCALE = (DH ** -0.5) * math.log2(math.e)
FLAG_LANE = 127


def _relayout(a, fill):
    rows = a.shape[0]
    lane = lax.broadcasted_iota(jnp.int32, (rows, 128), 1)
    parts = []
    for T in range(NT):
        t0, off = divmod(120 * T, 128)
        n = min(120, D - 120 * T)
        lo = a[:, 128 * t0:128 * (t0 + 1)]
        if off:
            sh = 128 - off
            v = pltpu.roll(lo, sh, 1)
            if n > sh:
                hi = pltpu.roll(a[:, 128 * (t0 + 1):128 * (t0 + 2)], sh, 1)
                v = jnp.where(lane < sh, v, hi)
        else:
            v = lo
        parts.append(jnp.where(lane < n, v, fill))
    return jnp.concatenate(parts, axis=1)


def _kernel(x_ref, wqkv_hbm, wo_hbm, w1_hbm, w2_hbm, gw_ref, o_ref,
            k_scr, vt_scr, wvt_scr, ot_scr, st_scr,
            wqkv_ref, wo_ref, w1_ref, w2_ref, sems):
    step = pl.program_id(0)
    copies = [pltpu.make_async_copy(src, dst, sems.at[i]) for i, (src, dst) in enumerate(
        [(wqkv_hbm, wqkv_ref), (wo_hbm, wo_ref), (w1_hbm, w1_ref), (w2_hbm, w2_ref)])]

    @pl.when(step == 0)
    def _init():
        for c in copies:
            c.start()
        lane = lax.broadcasted_iota(jnp.int32, (W, 128 * NT), 1) & 127
        pad = jnp.where(lane == FLAG_LANE, NEG, 0.0).astype(jnp.bfloat16)
        k_scr[0:W // 2, :] = pltpu.bitcast(pad, jnp.uint32)
        vt_scr[:, 0:W] = jnp.zeros((vt_scr.shape[0], W), vt_scr.dtype)
        copies[0].wait()
        wvt_scr[...] = wqkv_ref[:, 2 * D:3 * D].astype(jnp.float32).T.astype(jnp.bfloat16)

    x = x_ref[...]
    base = pl.multiple_of(step * BQ, BQ)

    qk = jnp.dot(x, wqkv_ref[:, 0:2 * D], preferred_element_type=jnp.float32)
    zero_fill = jnp.zeros((BQ, 128), jnp.float32)
    q = _relayout(qk[:, 0:D] * QSCALE, zero_fill)
    kk = _relayout(qk[:, D:2 * D], zero_fill).astype(jnp.bfloat16)
    k_scr[pl.ds(pl.multiple_of((base + W) // 2, BQ // 2), BQ // 2), :] = pltpu.bitcast(kk, jnp.uint32)
    vt = lax.dot_general(wvt_scr[...], x, (((1,), (1,)), ((), ())),
                         preferred_element_type=jnp.float32)
    tail = (lax.broadcasted_iota(jnp.int32, (VR - 40, BQ), 0) == 0).astype(jnp.float32)
    vt_parts = []
    for p in range(NP):
        vt_parts += [vt[40 * p:40 * p + 40, :], tail]
    vt_all = jnp.concatenate(vt_parts, axis=0).astype(jnp.bfloat16)
    vt_scr[:, pl.ds(base + W, BQ)] = pltpu.bitcast(vt_all, jnp.uint32)

    r64 = lax.broadcasted_iota(jnp.int32, (QB, 128), 0)
    lane_q = lax.broadcasted_iota(jnp.int32, (QB, 128), 1)
    upper = r64 > (lane_q & (QB - 1))
    flag_one = (lane_q == FLAG_LANE).astype(jnp.float32)
    lane40 = lax.broadcasted_iota(jnp.int32, (40, 128), 1)
    row40 = lax.broadcasted_iota(jnp.int32, (40, 128), 0)
    zpad = jnp.zeros((QB, 128), jnp.float32)

    for p in range(NP):
        t, off = p // 3, 40 * (p % 3)
        m_a = (lane_q >= off) & (lane_q < off + DH)
        m_b = (lane_q >= off + DH) & (lane_q < off + 2 * DH)
        for jj in range(NU):
            row0 = pl.multiple_of((base + QB * jj) // 2, QB // 2)
            kw = pltpu.bitcast(k_scr[pl.ds(row0, KW // 2), 128 * t:128 * (t + 1)], jnp.bfloat16)
            qt = q[QB * jj:QB * (jj + 1), 128 * t:128 * (t + 1)]
            qa = jnp.where(m_a, qt, flag_one)
            qb = jnp.where(m_b, qt, flag_one)
            qbd = jnp.concatenate([qa, qb] if jj % 2 == 0 else [qb, qa], axis=0).astype(jnp.bfloat16)
            st_scr[p * NU + jj] = lax.dot_general(
                kw, qbd, (((1,), (1,)), ((), ())), preferred_element_type=jnp.float32)
    for p in range(NP):
        outs = []
        for jj in range(NU):
            st = st_scr[p * NU + jj]
            top = jnp.where(upper, st[0:QB], st[W:KW])
            mid = st[QB:W]
            m = jnp.maximum(jnp.max(top, axis=0, keepdims=True),
                            jnp.max(mid, axis=0, keepdims=True))
            e_top = jnp.exp2(top - m)
            e_mid = jnp.exp2(mid - m)
            pieces = [jnp.where(upper, e_top, 0.0), e_mid, jnp.where(upper, 0.0, e_top)]
            if jj % 2 == 0:
                pt = jnp.concatenate(pieces + [zpad], axis=0)
            else:
                pt = jnp.concatenate([zpad] + pieces, axis=0)
            pt = pt.astype(jnp.bfloat16)
            col0 = pl.multiple_of(base + QB * (jj - jj % 2), 128)
            vw = pltpu.bitcast(vt_scr[VR // 2 * p:VR // 2 * (p + 1), pl.ds(col0, 384)], jnp.bfloat16)
            ot = jnp.dot(vw, pt, preferred_element_type=jnp.float32)
            outs.append(ot[0:40] * (1.0 / ot[40:41]))
        for u in range(NU // 2):
            o_e, o_o = outs[2 * u], outs[2 * u + 1]
            first = jnp.where(lane40 < QB, o_e, o_o)
            second = pltpu.roll(jnp.where(lane40 < QB, o_o, o_e), QB, 1)
            ot_scr[40 * p:40 * p + 40, 128 * u:128 * (u + 1)] = jnp.where(row40 < DH, first, second)

    @pl.when(step == 0)
    def _wait_rest():
        for c in copies[1:]:
            c.wait()

    o_att = ot_scr[...].T.astype(jnp.bfloat16)
    a = jnp.dot(o_att, wo_ref[...], preferred_element_type=jnp.float32)

    h = jnp.dot(x, w1_ref[...], preferred_element_type=jnp.float32)
    h = (h * jax.nn.sigmoid(h)).astype(jnp.bfloat16)
    b = jnp.dot(h, w2_ref[...], preferred_element_type=jnp.float32)

    z = jnp.sum(x.astype(jnp.float32) * gw_ref[...].astype(jnp.float32), axis=-1, keepdims=True)
    g = jax.nn.sigmoid(z)
    o_ref[...] = (g * a + (1.0 - g) * b).astype(o_ref.dtype)


@jax.jit
def pallas_gated_mix__sliding_block__dense_activation_silu__prompt_kernel(
    A_x, A_wqkv, A_wo, B_x, B_w1, B_w2, gate_w):
    del B_x
    x2 = A_x.reshape(S, D)
    gw = gate_w.reshape(1, D)
    const = lambda i: (0, 0)
    out = pl.pallas_call(
        _kernel,
        grid=(S // BQ,),
        in_specs=[
            pl.BlockSpec((BQ, D), lambda i: (i, 0)),
            pl.BlockSpec(memory_space=pl.ANY),
            pl.BlockSpec(memory_space=pl.ANY),
            pl.BlockSpec(memory_space=pl.ANY),
            pl.BlockSpec(memory_space=pl.ANY),
            pl.BlockSpec((1, D), const),
        ],
        out_specs=pl.BlockSpec((BQ, D), lambda i: (i, 0)),
        out_shape=jax.ShapeDtypeStruct((S, D), jnp.bfloat16),
        scratch_shapes=[
            pltpu.VMEM(((S + W) // 2, 128 * NT), jnp.uint32),
            pltpu.VMEM((VR * NP // 2, S + W), jnp.uint32),
            pltpu.VMEM((D, D), jnp.bfloat16),
            pltpu.VMEM((D, BQ), jnp.float32),
            pltpu.VMEM((NP * NU, KW, 128), jnp.float32),
            pltpu.VMEM((D, 3 * D), jnp.bfloat16),
            pltpu.VMEM((D, D), jnp.bfloat16),
            pltpu.VMEM((D, F), jnp.bfloat16),
            pltpu.VMEM((F, D), jnp.bfloat16),
            pltpu.SemaphoreType.DMA((4,)),
        ],
        compiler_params=pltpu.CompilerParams(
            dimension_semantics=("arbitrary",),
            vmem_limit_bytes=100 * 1024 * 1024),
    )(x2, A_wqkv, A_wo, B_w1, B_w2, gw)
    return out.reshape(1, S, D)
```

```python
import functools
import math

import jax
import jax.numpy as jnp
from jax import lax
from jax.experimental import pallas as pl
from jax.experimental.pallas import tpu as pltpu

S, D, F = 2048, 640, 1536
H, DH, W = 32, 20, 256
BQ = 256
QB = 64
NP = H // 2
NU = BQ // QB
KW = W + QB
NT = 6
NEG = -1e30
QSCALE = (DH ** -0.5) * math.log2(math.e)
FLAG_LANE = 127
ONES_WORD = 0x3F803F80


def _relayout(a, fill):
    rows = a.shape[0]
    lane = lax.broadcasted_iota(jnp.int32, (rows, 128), 1)
    parts = []
    for T in range(NT):
        t0, off = divmod(120 * T, 128)
        n = min(120, D - 120 * T)
        lo = a[:, 128 * t0:128 * (t0 + 1)]
        if off:
            sh = 128 - off
            v = pltpu.roll(lo, sh, 1)
            if n > sh:
                hi = pltpu.roll(a[:, 128 * (t0 + 1):128 * (t0 + 2)], sh, 1)
                v = jnp.where(lane < sh, v, hi)
        else:
            v = lo
        parts.append(jnp.where(lane < n, v, fill))
    return jnp.concatenate(parts, axis=1)


def _kernel(x_ref, wqkv_hbm, wo_hbm, w1_hbm, w2_hbm, gw_ref, o_ref,
            k_scr, vt_scr, wvt_scr, ot_scr, st_scr,
            wqkv_ref, wo_ref, w1_ref, w2_ref, sems):
    step = pl.program_id(0)
    copies = [pltpu.make_async_copy(src, dst, sems.at[i]) for i, (src, dst) in enumerate(
        [(wqkv_hbm.at[:, c * D:(c + 1) * D], wqkv_ref.at[:, c * D:(c + 1) * D]) for c in range(3)]
        + [(w1_hbm, w1_ref), (wo_hbm, wo_ref), (w2_hbm, w2_ref)])]

    def body(first):
        if first:
            for c in copies:
                c.start()
            lane = lax.broadcasted_iota(jnp.int32, (W, 128 * NT), 1) & 127
            pad = jnp.where(lane == FLAG_LANE, NEG, 0.0).astype(jnp.bfloat16)
            k_scr[0:W // 2, :] = pltpu.bitcast(pad, jnp.uint32)
            vt_scr[:, 0:W] = jnp.zeros((vt_scr.shape[0], W), vt_scr.dtype)
            copies[0].wait()

        x = x_ref[...]
        base = pl.multiple_of(step * BQ, BQ)

        zero_fill = jnp.zeros((BQ, 128), jnp.float32)
        if first:
            qn = jnp.dot(x, wqkv_ref[:, 0:D], preferred_element_type=jnp.float32)
            copies[1].wait()
            kn = jnp.dot(x, wqkv_ref[:, D:2 * D], preferred_element_type=jnp.float32)
            copies[2].wait()
            wvt_scr[...] = wqkv_ref[:, 2 * D:3 * D].astype(jnp.float32).T.astype(jnp.bfloat16)
        else:
            qk = jnp.dot(x, wqkv_ref[:, 0:2 * D], preferred_element_type=jnp.float32)
            qn, kn = qk[:, 0:D], qk[:, D:2 * D]
        q = _relayout(qn * QSCALE, zero_fill)
        kk = _relayout(kn, zero_fill).astype(jnp.bfloat16)
        k_scr[pl.ds(pl.multiple_of((base + W) // 2, BQ // 2), BQ // 2), :] = pltpu.bitcast(kk, jnp.uint32)
        vt = lax.dot_general(wvt_scr[...], x, (((1,), (1,)), ((), ())),
                             preferred_element_type=jnp.float32)
        vt_scr[:, pl.ds(base + W, BQ)] = pltpu.bitcast(vt.astype(jnp.bfloat16), jnp.uint32)

        r64 = lax.broadcasted_iota(jnp.int32, (QB, 128), 0)
        lane_q = lax.broadcasted_iota(jnp.int32, (QB, 128), 1)
        upper = r64 > (lane_q & (QB - 1))
        flag_one = (lane_q == FLAG_LANE).astype(jnp.float32)
        left192 = lax.broadcasted_iota(jnp.int32, (192, 128), 1) < QB
        wrow16 = lax.broadcasted_iota(jnp.int32, (16, 384), 0)
        row8 = lax.broadcasted_iota(jnp.int32, (8, 128), 0)
        zpad = jnp.zeros((QB, 128), jnp.float32)

        for p in range(NP):
            t, off = p // 3, 40 * (p % 3)
            m_a = (lane_q >= off) & (lane_q < off + DH)
            m_b = (lane_q >= off + DH) & (lane_q < off + 2 * DH)
            for u in range(NU // 2):
                row0 = pl.multiple_of((base + 128 * u) // 2, 64)
                kw = pltpu.bitcast(k_scr[pl.ds(row0, 192), 128 * t:128 * (t + 1)], jnp.bfloat16)
                qe = q[128 * u:128 * u + QB, 128 * t:128 * (t + 1)]
                qo = q[128 * u + QB:128 * (u + 1), 128 * t:128 * (t + 1)]
                qae, qbe = jnp.where(m_a, qe, flag_one), jnp.where(m_b, qe, flag_one)
                qao, qbo = jnp.where(m_a, qo, flag_one), jnp.where(m_b, qo, flag_one)
                nt = (((1,), (1,)), ((), ()))
                idx = p * (NU // 2) + u

                def sc(rows, blocks):
                    return lax.dot_general(rows, jnp.concatenate(blocks, axis=0).astype(jnp.bfloat16),
                                           nt, preferred_element_type=jnp.float32)
                st_scr[idx, 0:256] = sc(kw[64:320], [qae, qao])
                st_scr[idx, 256:512] = sc(kw[64:320], [qbo, qbe])
                st_scr[idx, 512:576] = sc(kw[0:64], [qae, qbe])
                st_scr[idx, 576:640] = sc(kw[320:384], [qbo, qao])

        def head_out(h, pt, col0):
            start = (DH * h // 16) * 16
            o = DH * h - start
            ones_at = 0 if o >= 4 else 15
            vw = vt_scr[start // 2:start // 2 + 16, pl.ds(col0, 384)]
            vw = jnp.where(wrow16 == ones_at, jnp.uint32(ONES_WORD), vw)
            res = jnp.dot(pltpu.bitcast(vw, jnp.bfloat16), pt.astype(jnp.bfloat16),
                          preferred_element_type=jnp.float32)
            inv = 1.0 / res[2 * ones_at:2 * ones_at + 1]
            lo = (o // 8) * 8
            return res[lo:lo + 24] * inv

        left64 = lane_q < QB
        mask_e = [left64 & upper, upper & ~left64]
        mask_o = [~(left64 | upper), left64 & ~upper]
        for p in range(NP):
            for u in range(NU // 2):
                col0 = pl.multiple_of(base + 128 * u, 128)
                s_ref = st_scr.at[p * (NU // 2) + u]
                rs = []
                for hh in range(2):
                    o = 256 * hh
                    m0 = jnp.where(mask_o[hh], s_ref[576:640], s_ref[o:o + 64])
                    m1 = s_ref[o + 64:o + 192]
                    m2 = jnp.where(mask_e[hh], s_ref[512:576], s_ref[o + 192:o + 256])
                    m = jnp.max(jnp.concatenate([m0, m1, m2], axis=0), axis=0, keepdims=True)
                    e0, e1, e2 = jnp.exp2(m0 - m), jnp.exp2(m1 - m), jnp.exp2(m2 - m)
                    pt = jnp.concatenate([jnp.where(mask_e[hh], e2, 0.0), jnp.where(mask_o[hh], 0.0, e0), e1,
                                          jnp.where(mask_e[hh], 0.0, e2), jnp.where(mask_o[hh], e0, 0.0)], axis=0)
                    rs.append(head_out(2 * p + hh, pt, col0))
                ra, rb = rs[0], pltpu.roll(rs[1], QB, 1)
                blk = jnp.concatenate(
                    [ra[0:16], jnp.where(row8 < 4, ra[16:24], rb[0:8]), rb[8:24]], axis=0)
                ot_scr[40 * p:40 * p + 40, 128 * u:128 * (u + 1)] = blk

        if first:
            for c in copies[3:]:
                c.wait()

        h = jnp.dot(x, w1_ref[...], preferred_element_type=jnp.float32)
        h = (h * jax.nn.sigmoid(h)).astype(jnp.bfloat16)
        o_att = ot_scr[...].T.astype(jnp.bfloat16)
        a = jnp.dot(o_att, wo_ref[...], preferred_element_type=jnp.float32)
        b = jnp.dot(h, w2_ref[...], preferred_element_type=jnp.float32)

        z = jnp.sum(x.astype(jnp.float32) * gw_ref[...].astype(jnp.float32).reshape(1, D), axis=-1, keepdims=True)
        g = jax.nn.sigmoid(z)
        o_ref[...] = (g * a + (1.0 - g) * b).astype(o_ref.dtype)

    pl.when(step == 0)(lambda: body(True))
    pl.when(step != 0)(lambda: body(False))


@jax.jit
def pallas_gated_mix__sliding_block__dense_activation_silu__prompt_kernel(
    A_x, A_wqkv, A_wo, B_x, B_w1, B_w2, gate_w):
    del B_x
    x2 = A_x.reshape(S, D)
    const = lambda i: (0, 0)
    out = pl.pallas_call(
        _kernel,
        grid=(S // BQ,),
        in_specs=[
            pl.BlockSpec((BQ, D), lambda i: (i, 0)),
            pl.BlockSpec(memory_space=pl.ANY),
            pl.BlockSpec(memory_space=pl.ANY),
            pl.BlockSpec(memory_space=pl.ANY),
            pl.BlockSpec(memory_space=pl.ANY),
            pl.BlockSpec((D,), lambda i: (0,)),
        ],
        out_specs=pl.BlockSpec((BQ, D), lambda i: (i, 0)),
        out_shape=jax.ShapeDtypeStruct((S, D), jnp.bfloat16),
        scratch_shapes=[
            pltpu.VMEM(((S + W) // 2, 128 * NT), jnp.uint32),
            pltpu.VMEM((D // 2, S + W), jnp.uint32),
            pltpu.VMEM((D, D), jnp.bfloat16),
            pltpu.VMEM((D, BQ), jnp.float32),
            pltpu.VMEM((NP * NU // 2, 640, 128), jnp.float32),
            pltpu.VMEM((D, 3 * D), jnp.bfloat16),
            pltpu.VMEM((D, D), jnp.bfloat16),
            pltpu.VMEM((D, F), jnp.bfloat16),
            pltpu.VMEM((F, D), jnp.bfloat16),
            pltpu.SemaphoreType.DMA((6,)),
        ],
        compiler_params=pltpu.CompilerParams(
            dimension_semantics=("arbitrary",),
            vmem_limit_bytes=100 * 1024 * 1024),
    )(x2, A_wqkv, A_wo, B_w1, B_w2, gate_w)
    return out.reshape(1, S, D)
```

```python
import math

import jax
import jax.numpy as jnp
from jax import lax
from jax.experimental import pallas as pl
from jax.experimental.pallas import tpu as pltpu

S, D, F = 2048, 640, 1536
H, DH, W = 32, 20, 256
BQ = 256
NB = BQ // 128
NP = H // 2
NT = 6
NEG = -1e30
QSCALE = (DH ** -0.5) * math.log2(math.e)
ONES_WORD = 0x3F803F80
_NT_DIMS = (((1,), (1,)), ((), ()))


def _relayout(a):
    rows = a.shape[0]
    lane = lax.broadcasted_iota(jnp.int32, (rows, 128), 1)
    parts = []
    for t in range(NT):
        t0, off = divmod(120 * t, 128)
        n = min(120, D - 120 * t)
        v = a[:, 128 * t0:128 * (t0 + 1)]
        if off:
            sh = 128 - off
            v = pltpu.roll(v, sh, 1)
            if n > sh:
                hi = pltpu.roll(a[:, 128 * (t0 + 1):128 * (t0 + 2)], sh, 1)
                v = jnp.where(lane < sh, v, hi)
        parts.append(jnp.where(lane < n, v, 0.0))
    return jnp.concatenate(parts, axis=1)


def _kernel(x_ref, wqkv_hbm, wo_hbm, w1_hbm, w2_hbm, gw_ref, o_ref,
            k_scr, vt_scr, wvt_scr, ot_scr, st_scr,
            wqkv_ref, wo_ref, w1_ref, w2_ref, sems):
    step = pl.program_id(0)
    copies = [pltpu.make_async_copy(src, dst, sems.at[i]) for i, (src, dst) in enumerate(
        [(wqkv_hbm.at[:, c * D:(c + 1) * D], wqkv_ref.at[:, c * D:(c + 1) * D]) for c in range(3)]
        + [(w1_hbm, w1_ref), (w2_hbm, w2_ref), (wo_hbm, wo_ref)])]

    def body(first):
        if first:
            for c in copies:
                c.start()
            copies[0].wait()

        x = x_ref[...]
        base = pl.multiple_of(step * BQ, BQ)

        if first:
            qn = jnp.dot(x, wqkv_ref[:, 0:D], preferred_element_type=jnp.float32)
            copies[1].wait()
            kn = jnp.dot(x, wqkv_ref[:, D:2 * D], preferred_element_type=jnp.float32)
            copies[2].wait()
            wvt_scr[...] = wqkv_ref[:, 2 * D:3 * D].astype(jnp.float32).T.astype(jnp.bfloat16)
        else:
            qk = jnp.dot(x, wqkv_ref[:, 0:2 * D], preferred_element_type=jnp.float32)
            qn, kn = qk[:, 0:D], qk[:, D:2 * D]
        q = _relayout(qn * QSCALE)
        kk = _relayout(kn).astype(jnp.bfloat16)
        k_scr[pl.ds(pl.multiple_of(base // 2, BQ // 2), BQ // 2), :] = pltpu.bitcast(kk, jnp.uint32)
        vt = lax.dot_general(wvt_scr[...], x, _NT_DIMS,
                             preferred_element_type=jnp.float32)
        vt_scr[:, pl.ds(base, BQ)] = pltpu.bitcast(vt.astype(jnp.bfloat16), jnp.uint32)

        row = lax.broadcasted_iota(jnp.int32, (64, 128), 0)
        lane = lax.broadcasted_iota(jnp.int32, (64, 128), 1)
        upper = row > (lane & 63)
        left = lane < 64
        mask_e = [left & upper, upper & ~left]
        mask_o = [~(left | upper), left & ~upper]
        row8 = lax.broadcasted_iota(jnp.int32, (8, 128), 0)

        def n_invalid(u):
            return W - 128 * u if first else 0

        for p in range(NP):
            t, off = p // 3, 40 * (p % 3)
            m_a = (lane >= off) & (lane < off + DH)
            m_b = (lane >= off + DH) & (lane < off + 2 * DH)
            for u in range(NB):
                nv = n_invalid(u)
                lo = max(nv, 64)
                row0 = pl.multiple_of((base + 128 * u - W + nv) // 2, 64)
                kw = pltpu.bitcast(
                    k_scr[pl.ds(row0, (384 - nv) // 2), 128 * t:128 * (t + 1)], jnp.bfloat16)
                qe = q[128 * u:128 * u + 64, 128 * t:128 * (t + 1)]
                qo = q[128 * u + 64:128 * (u + 1), 128 * t:128 * (t + 1)]
                qae, qbe = jnp.where(m_a, qe, 0.0), jnp.where(m_b, qe, 0.0)
                qao, qbo = jnp.where(m_a, qo, 0.0), jnp.where(m_b, qo, 0.0)
                idx = p * NB + u

                def sc(r0, r1, blocks):
                    return lax.dot_general(
                        kw[r0 - nv:r1 - nv], jnp.concatenate(blocks, axis=0).astype(jnp.bfloat16),
                        _NT_DIMS, preferred_element_type=jnp.float32)
                st_scr[idx, lo - 64:256] = sc(lo, 320, [qae, qao])
                st_scr[idx, 256 + lo - 64:512] = sc(lo, 320, [qbo, qbe])
                if nv == 0:
                    st_scr[idx, 512:576] = sc(0, 64, [qae, qbe])
                st_scr[idx, 576:640] = sc(320, 384, [qbo, qao])

        pts = {}
        for p in range(NP):
            for u in range(NB):
                nv = n_invalid(u)
                s_ref = st_scr.at[p * NB + u]
                for hh in range(2):
                    o = 256 * hh
                    m0 = jnp.where(mask_o[hh], s_ref[576:640], s_ref[o:o + 64] if nv == 0 else NEG)
                    m2 = jnp.where(mask_e[hh], s_ref[512:576] if nv == 0 else NEG,
                                   s_ref[o + 192:o + 256])
                    ms = [m0, s_ref[o + 64:o + 192], m2] if nv < 256 else [m0, m2]
                    m = jnp.max(jnp.concatenate(ms, axis=0), axis=0, keepdims=True)
                    es = [jnp.exp2(v - m) for v in ms]
                    e0, e2 = es[0], es[-1]
                    pieces = []
                    if nv == 0:
                        pieces += [jnp.where(mask_e[hh], e2, 0.0), jnp.where(mask_o[hh], 0.0, e0)]
                    if nv < 256:
                        pieces += [es[1]]
                    pieces += [jnp.where(mask_e[hh], 0.0, e2), jnp.where(mask_o[hh], e0, 0.0)]
                    pts[(2 * p + hh, u)] = jnp.concatenate(pieces, axis=0).astype(jnp.bfloat16)

        if first:
            copies[3].wait()
        h = jnp.dot(x, w1_ref[...], preferred_element_type=jnp.float32)
        h = (h * jax.nn.sigmoid(h)).astype(jnp.bfloat16)

        def head_out(hd, u):
            nv = n_invalid(u)
            start = (DH * hd // 16) * 16
            o = DH * hd - start
            ones_at = 0 if o >= 4 else 15
            col0 = pl.multiple_of(base + 128 * u - W + nv, 128)
            vw = vt_scr[start // 2:start // 2 + 16, pl.ds(col0, 384 - nv)]
            wrow = lax.broadcasted_iota(jnp.int32, (16, 384 - nv), 0)
            vw = jnp.where(wrow == ones_at, jnp.uint32(ONES_WORD), vw)
            res = jnp.dot(pltpu.bitcast(vw, jnp.bfloat16), pts[(hd, u)],
                          preferred_element_type=jnp.float32)
            inv = 1.0 / res[2 * ones_at:2 * ones_at + 1]
            lo = (o // 8) * 8
            return res[lo:lo + 24] * inv

        for p in range(NP):
            for u in range(NB):
                ra = head_out(2 * p, u)
                rb = pltpu.roll(head_out(2 * p + 1, u), 64, 1)
                ot_scr[40 * p:40 * p + 40, 128 * u:128 * (u + 1)] = jnp.concatenate(
                    [ra[0:16], jnp.where(row8 < 4, ra[16:24], rb[0:8]), rb[8:24]], axis=0)

        if first:
            copies[4].wait()
            copies[5].wait()
        b = jnp.dot(h, w2_ref[...], preferred_element_type=jnp.float32)
        o_att = ot_scr[...].T.astype(jnp.bfloat16)
        a = jnp.dot(o_att, wo_ref[...], preferred_element_type=jnp.float32)

        gw = gw_ref[...].astype(jnp.float32).reshape(1, D)
        g = jax.nn.sigmoid(jnp.sum(x.astype(jnp.float32) * gw, axis=-1, keepdims=True))
        o_ref[...] = (g * a + (1.0 - g) * b).astype(o_ref.dtype)

    pl.when(step == 0)(lambda: body(True))
    pl.when(step != 0)(lambda: body(False))


@jax.jit
def pallas_gated_mix__sliding_block__dense_activation_silu__prompt_kernel(
    A_x, A_wqkv, A_wo, B_x, B_w1, B_w2, gate_w):
    del B_x
    out = pl.pallas_call(
        _kernel,
        grid=(S // BQ,),
        in_specs=[
            pl.BlockSpec((BQ, D), lambda i: (i, 0)),
            pl.BlockSpec(memory_space=pl.ANY),
            pl.BlockSpec(memory_space=pl.ANY),
            pl.BlockSpec(memory_space=pl.ANY),
            pl.BlockSpec(memory_space=pl.ANY),
            pl.BlockSpec((D,), lambda i: (0,)),
        ],
        out_specs=pl.BlockSpec((BQ, D), lambda i: (i, 0)),
        out_shape=jax.ShapeDtypeStruct((S, D), jnp.bfloat16),
        scratch_shapes=[
            pltpu.VMEM((S // 2, 128 * NT), jnp.uint32),
            pltpu.VMEM((D // 2, S), jnp.uint32),
            pltpu.VMEM((D, D), jnp.bfloat16),
            pltpu.VMEM((D, BQ), jnp.float32),
            pltpu.VMEM((NP * NB, 640, 128), jnp.float32),
            pltpu.VMEM((D, 3 * D), jnp.bfloat16),
            pltpu.VMEM((D, D), jnp.bfloat16),
            pltpu.VMEM((D, F), jnp.bfloat16),
            pltpu.VMEM((F, D), jnp.bfloat16),
            pltpu.SemaphoreType.DMA((6,)),
        ],
        compiler_params=pltpu.CompilerParams(
            dimension_semantics=("arbitrary",),
            vmem_limit_bytes=100 * 1024 * 1024),
    )(A_x.reshape(S, D), A_wqkv, A_wo, B_w1, B_w2, gate_w)
    return out.reshape(1, S, D)
```
